```python
import jax
import jax.numpy as jnp

def _softmax(x, axis=-1):
    return jax.nn.softmax(x, axis=axis)
def _gelu(x):
    return jax.nn.gelu(x, approximate=True)
def _silu(x):
    return jax.nn.silu(x)
def _sigmoid(x):
    return jax.nn.sigmoid(x)
def _layernorm(x, axis=-1, eps=1e-5):
    m = jnp.mean(x, axis=axis, keepdims=True)
    v = jnp.var(x, axis=axis, keepdims=True)
    return (x - m) / jnp.sqrt(v + eps)
def _scatter_add(tgt, idx, src, axis=0):
    return tgt.at[idx].add(src)
def _segment_sum(src, seg, n):
    return jax.ops.segment_sum(src, seg, n)
class _Rng:
    def __init__(self, key):
        self._k = key
    def _next(self):
        self._k, sub = jax.random.split(self._k)
        return sub
    def normal(self, shape):
        return jax.random.normal(self._next(), shape, dtype=jnp.bfloat16)
    def randint(self, lo, hi, shape):
        return jax.random.randint(self._next(), shape, lo, hi, dtype=jnp.int32)
    def uniform(self, shape, lo=0.0, hi=1.0):
        return jax.random.uniform(self._next(), shape, jnp.bfloat16, lo, hi)
    def permutation(self, n):
        return jax.random.permutation(self._next(), n)


kernel_name = 'recurrent_scan__gqa_block_cached__geglu_ffn__decode'

def _fwd_setup_inputs():
    _rng = _Rng(jax.random.key(int.from_bytes(__import__("os").urandom(4), "little")))
    _w = (lambda a: (lambda t: t.astype(jnp.bfloat16) if jnp.issubdtype(t.dtype, jnp.floating) else t)(jnp.asarray(a)))
    def _A_setup():
        B, Sq, D = 1, 1, 512
        Hq, Hkv, Sk, Dh = 32, 32, 4096, 128
        assert Hq % Hkv == 0, (Hq, Hkv)
        return {
            "x": _w((lambda *s: _rng.normal(s) * 0.05)(B, Sq, D)),
            "k_cache": _w((lambda *s: _rng.normal(s) * 0.05)(B, Hkv, Sk, Dh)),
            "v_cache": _w((lambda *s: _rng.normal(s) * 0.05)(B, Hkv, Sk, Dh)),
            "wq": _w((lambda *s: _rng.normal(s) * 0.05)(D, Hq * Dh) * (D ** -0.5)),
            "wo": _w((lambda *s: _rng.normal(s) * 0.05)(Hq * Dh, D) * ((Hq * Dh) ** -0.5)),
        }
    _A_in = _A_setup()

    def _B_setup():
        B, S, D, F = 1, 1, 512, 1376
        return {
            "x": _w((lambda *s: _rng.normal(s) * 0.05)(B, S, D)),
            "w_gate": _w((lambda *s: _rng.normal(s) * 0.05)(D, F)),
            "w_up": _w((lambda *s: _rng.normal(s) * 0.05)(D, F)),
            "w_down": _w((lambda *s: _rng.normal(s) * 0.05)(F, D)),
        }
    _B_in = _B_setup()

    return {
        "A_x": _A_in["x"],
        "A_k_cache": _A_in["k_cache"],
        "A_v_cache": _A_in["v_cache"],
        "A_wq": _A_in["wq"],
        "A_wo": _A_in["wo"],
        "B_x": _B_in["x"],
        "B_w_gate": _B_in["w_gate"],
        "B_w_up": _B_in["w_up"],
        "B_w_down": _B_in["w_down"],
    }

def _fwd_reference(A_x, A_k_cache, A_v_cache, A_wq, A_wo, B_x, B_w_gate, B_w_up, B_w_down):
    def _A_ref(x, k_cache, v_cache, wq, wo):
        B, Sq, D = x.shape
        Hq, Dh = 32, 128
        Hkv = k_cache.shape[1]
        rep = Hq // Hkv
        q = (lambda x, *d: x.transpose(*d))((x @ wq).reshape(B, Sq, Hq, Dh), 0, 2, 1, 3)
        k = jnp.repeat(k_cache, rep, axis=1)
        v = jnp.repeat(v_cache, rep, axis=1)
        scores = jnp.einsum("bhqd,bhkd->bhqk", q, k) * (Dh ** -0.5)
        p = _softmax(scores, axis=-1)
        o = jnp.einsum("bhqk,bhkd->bhqd", p, v)
        return (lambda x, *d: x.transpose(*d))(o, 0, 2, 1, 3).reshape(B, Sq, Hq * Dh) @ wo

    def _B_ref(x, w_gate, w_up, w_down):
        return (_gelu(x @ w_gate) * (x @ w_up)) @ w_down

    x = A_x
    xn = _layernorm(x, axis=-1)
    s = _A_ref(xn, A_k_cache, A_v_cache, A_wq, A_wo)
    g = _silu(_B_ref(xn, B_w_gate, B_w_up, B_w_down))
    return x + s * g


def setup_inputs():
    _inp = _fwd_setup_inputs()
    _gk = jax.random.fold_in(jax.random.key(int.from_bytes(__import__("os").urandom(4), "little")), 2**31 - 1)
    _shapes = [[1, 1, 512]]
    _dtypes = ['bfloat16']
    _gks = jax.random.split(_gk, len(_shapes))
    _gs = [jax.random.normal(k, s, dtype=jnp.dtype(d)) * 0.05 for k, s, d in zip(_gks, _shapes, _dtypes)]
    _inp["grad_out"] = _gs[0]
    return _inp

def reference(A_x, A_k_cache, A_v_cache, A_wq, A_wo, B_w_gate, B_w_up, B_w_down, B_x, grad_out):
    _const = dict(B_x=B_x)
    def _f(*_d):
        return _fwd_reference(**{'A_x': _d[0], 'A_k_cache': _d[1], 'A_v_cache': _d[2], 'A_wq': _d[3], 'A_wo': _d[4], 'B_w_gate': _d[5], 'B_w_up': _d[6], 'B_w_down': _d[7], **_const})
    _out, _vjp = jax.vjp(_f, A_x, A_k_cache, A_v_cache, A_wq, A_wo, B_w_gate, B_w_up, B_w_down)
    _grads = _vjp(grad_out)
    _out0 = jnp.asarray(_out)
    return (_out0, *[jnp.asarray(_g) for _g in _grads])
```

```python
import jax
import jax.numpy as jnp
import jax.experimental.pallas as pl
import jax.experimental.pallas.tpu as pltpu

F32 = jnp.float32
BF16 = jnp.bfloat16
LANES = 128
ROWS = 8
LN_EPS = 1e-5
GELU_C = 0.7978845608028654
GELU_A = 0.044715

READ_AHEAD = 4
WRITE_HEADS = 8
WRITE_ROWS = 64
PRIMED_WRITES = 64


def _nn(a, b):
    return jax.lax.dot_general(
        a, b, (((1,), (0,)), ((), ())), preferred_element_type=F32
    )


def _nt(a, b):
    return jax.lax.dot_general(
        a, b, (((1,), (1,)), ((), ())), preferred_element_type=F32
    )


def _column(row):
    return jnp.broadcast_to(row[0:1], (LANES, LANES)).T


def _bf16_rounded(v):
    return v.astype(BF16).astype(F32)


def _gelu_and_grad(z):
    t = jnp.tanh(GELU_C * (z + GELU_A * z * z * z))
    cdf = 0.5 * (1.0 + t)
    pdf = 0.5 * (1.0 - t * t) * GELU_C * (1.0 + 3.0 * GELU_A * z * z)
    return z * cdf, cdf + z * pdf


def _kernel(
    x_hbm, k_hbm, v_hbm, wq_hbm, wo_hbm, wg_hbm, wu_hbm, wd_hbm, go_hbm,
    out_hbm, dx_hbm, dk_hbm, dv_hbm, dwq_hbm, dwo_hbm, dwg_hbm, dwu_hbm, dwd_hbm,
    k_buf, v_buf, wq_buf, wo_buf, wg_buf, wu_buf, wd_buf,
    x_buf, go_buf, out_buf, dx_buf, gate_buf, up_buf, xcol_buf,
    k_sem, v_sem, in_sem, out_sem,
):
    heads, seq, head_dim = k_buf.shape
    d_model = wq_buf.shape[0]
    d_ff = wg_hbm.shape[0]
    ff_tiles = wg_buf.shape[0] // LANES
    scale = head_dim ** -0.5

    def kv_reads(h):
        return (
            pltpu.make_async_copy(k_hbm.at[0, h], k_buf.at[h], k_sem.at[h]),
            pltpu.make_async_copy(v_hbm.at[0, h], v_buf.at[h], v_sem.at[h]),
        )

    ff_rows = pl.ds(0, d_ff)
    reads = [
        pltpu.make_async_copy(wg_hbm, wg_buf.at[ff_rows], in_sem.at[0]),
        pltpu.make_async_copy(x_hbm, x_buf, in_sem.at[1]),
        pltpu.make_async_copy(go_hbm, go_buf, in_sem.at[2]),
        pltpu.make_async_copy(wu_hbm, wu_buf.at[ff_rows], in_sem.at[3]),
        pltpu.make_async_copy(wd_hbm, wd_buf.at[ff_rows], in_sem.at[4]),
        pltpu.make_async_copy(wq_hbm, wq_buf, in_sem.at[5]),
        pltpu.make_async_copy(wo_hbm, wo_buf, in_sem.at[6]),
    ]
    for c in reads:
        c.start()
    for h in range(READ_AHEAD):
        for c in kv_reads(h):
            c.start()
    wg_read, x_read, go_read, wu_read, wd_read, wq_read, wo_read = reads

    ff_pad = wg_buf.shape[0] - d_ff
    if ff_pad:
        for buf in (wg_buf, wu_buf, wd_buf):
            buf[pl.ds(d_ff, ff_pad), :] = jnp.zeros((ff_pad, d_model), BF16)

    x_read.wait()
    go_read.wait()
    x = jnp.broadcast_to(x_buf[0].astype(F32), (ROWS, d_model))
    go = jnp.broadcast_to(go_buf[0].astype(F32), (ROWS, d_model))
    xc = x - jnp.mean(x, axis=-1, keepdims=True)
    rstd = jax.lax.rsqrt(jnp.mean(xc * xc, axis=-1, keepdims=True) + LN_EPS)
    xn = xc * rstd
    xn_b = xn.astype(BF16)
    xn_r = xn_b.astype(F32)
    for t in range(d_model // LANES):
        cols = slice(t * LANES, (t + 1) * LANES)
        xcol_buf[cols, :] = _column(xn_r[:, cols])

    wg_read.wait()
    wu_read.wait()
    wd_read.wait()

    def ffn_fwd(t, b):
        rows = pl.ds(pl.multiple_of(t * LANES, LANES), LANES)
        gate = _nt(xn_b, wg_buf[rows, :])
        up = _nt(xn_b, wu_buf[rows, :])
        gate_buf[t] = gate
        up_buf[t] = up
        act, _ = _gelu_and_grad(gate)
        return b + _nn((act * up).astype(BF16), wd_buf[rows, :])

    b = jax.lax.fori_loop(0, ff_tiles, ffn_fwd, jnp.zeros((ROWS, d_model), F32))
    sig = jax.nn.sigmoid(b)
    g = b * sig
    ds_b = (go * g).astype(BF16)
    ds_r = ds_b.astype(F32)

    wq_read.wait()
    wo_read.wait()
    eye = jax.lax.broadcasted_iota(
        jnp.int32, (LANES, LANES), 0
    ) == jax.lax.broadcasted_iota(jnp.int32, (LANES, LANES), 1)

    def outer_into(buf, h, col_vec, row_vec):
        rhs = jnp.broadcast_to(row_vec[0:1], (LANES, head_dim)).astype(BF16)
        for t in range(seq // LANES):
            rows = slice(t * LANES, (t + 1) * LANES)
            tile = jnp.broadcast_to(col_vec[0:1, rows], (LANES, LANES))
            lhs = jnp.where(eye, tile, 0.0).astype(BF16)
            buf[h, rows, :] = _nn(lhs, rhs).astype(BF16)

    def head(h, carry):
        s_acc, dxn_acc = carry
        span = pl.ds(pl.multiple_of(h * head_dim, head_dim), head_dim)
        wq_h = wq_buf[:, span]
        wo_h = wo_buf[span, :]
        q = _nn(xn_b, wq_h)
        do = _nt(ds_b, wo_h)
        k_read, v_read = kv_reads(h)

        k_read.wait()
        scores = _nt(q.astype(BF16), k_buf[h]) * scale
        e = jnp.exp(scores - jnp.max(scores, axis=-1, keepdims=True))
        p = e / jnp.sum(e, axis=-1, keepdims=True)

        v_read.wait()
        dp = _nt(do.astype(BF16), v_buf[h])
        o = _nn(p.astype(BF16), v_buf[h])
        dsc = p * (dp - jnp.sum(p * dp, axis=-1, keepdims=True)) * scale
        dq = _nn(dsc.astype(BF16), k_buf[h])

        s_acc = s_acc + _nn(o.astype(BF16), wo_h)
        dxn_acc = dxn_acc + _nt(dq.astype(BF16), wq_h)

        outer_into(v_buf, h, p, do)
        outer_into(k_buf, h, dsc, q)
        wq_buf[:, span] = (xcol_buf[...] * _bf16_rounded(dq)[0:1]).astype(BF16)
        o_col = _column(_bf16_rounded(o))
        for t in range(d_model // LANES):
            cols = slice(t * LANES, (t + 1) * LANES)
            wo_buf[span, cols] = (o_col * ds_r[0:1, cols]).astype(BF16)
        return s_acc, dxn_acc

    row_blocks = seq // WRITE_ROWS
    kv_steps = (heads // WRITE_HEADS) * row_blocks

    def kv_write(src, dst, sem, i):
        hs = pl.ds((i // row_blocks) * WRITE_HEADS, WRITE_HEADS)
        rs = pl.ds(pl.multiple_of((i % row_blocks) * WRITE_ROWS, WRITE_ROWS), WRITE_ROWS)
        return pltpu.make_async_copy(src.at[hs, rs], dst.at[0, hs, rs], sem)

    def start_writes(src, dst, sem, lo, hi):
        def body(i, _):
            kv_write(src, dst, sem, i).start()
        jax.lax.fori_loop(lo, hi, body, None)

    def head_step(h, carry):
        @pl.when(h + READ_AHEAD < heads)
        def _():
            for c in kv_reads(h + READ_AHEAD):
                c.start()

        carry = head(h, carry)

        @pl.when(h == heads - 2)
        def _():
            start_writes(v_buf, dv_hbm, out_sem.at[0], 0, PRIMED_WRITES)

        return carry

    zeros = jnp.zeros((ROWS, d_model), F32)
    s, dxn = jax.lax.fori_loop(0, heads, head_step, (zeros, zeros))

    out_buf[0] = (x + s * g)[0:1].astype(BF16)
    db_b = ((go * s) * (sig * (1.0 + b * (1.0 - sig)))).astype(BF16)
    db_r = db_b.astype(F32)

    def ffn_bwd(t, acc):
        rows = pl.ds(pl.multiple_of(t * LANES, LANES), LANES)
        up = up_buf[t]
        act, act_grad = _gelu_and_grad(gate_buf[t])
        dh = _nt(db_b, wd_buf[rows, :])
        dgate = (dh * up * act_grad).astype(BF16)
        dup = (dh * act).astype(BF16)
        acc = acc + _nn(dgate, wg_buf[rows, :]) + _nn(dup, wu_buf[rows, :])
        for buf, col_vec, row_vec in (
            (wg_buf, dgate.astype(F32), xn_r),
            (wu_buf, dup.astype(F32), xn_r),
            (wd_buf, _bf16_rounded(act * up), db_r),
        ):
            col = _column(col_vec)
            for c in range(d_model // LANES):
                cols = slice(c * LANES, (c + 1) * LANES)
                buf[rows, cols] = (col * row_vec[0:1, cols]).astype(BF16)
        return acc

    dxn = jax.lax.fori_loop(0, ff_tiles, ffn_bwd, dxn)
    dx = go + rstd * (
        dxn
        - jnp.mean(dxn, axis=-1, keepdims=True)
        - xn * jnp.mean(dxn * xn, axis=-1, keepdims=True)
    )
    dx_buf[0] = dx[0:1].astype(BF16)

    small_writes = [
        pltpu.make_async_copy(out_buf, out_hbm, out_sem.at[2]),
        pltpu.make_async_copy(dx_buf, dx_hbm, out_sem.at[3]),
        pltpu.make_async_copy(wq_buf, dwq_hbm, out_sem.at[4]),
        pltpu.make_async_copy(wo_buf, dwo_hbm, out_sem.at[5]),
        pltpu.make_async_copy(wg_buf.at[ff_rows], dwg_hbm, out_sem.at[6]),
        pltpu.make_async_copy(wu_buf.at[ff_rows], dwu_hbm, out_sem.at[7]),
        pltpu.make_async_copy(wd_buf.at[ff_rows], dwd_hbm, out_sem.at[8]),
    ]
    for c in small_writes:
        c.start()
    start_writes(v_buf, dv_hbm, out_sem.at[0], PRIMED_WRITES, kv_steps)
    start_writes(k_buf, dk_hbm, out_sem.at[1], 0, kv_steps)

    for c in small_writes:
        c.wait()
    pltpu.make_async_copy(v_buf, dv_hbm.at[0], out_sem.at[0]).wait()
    pltpu.make_async_copy(k_buf, dk_hbm.at[0], out_sem.at[1]).wait()


@jax.jit
def pallas_recurrent_scan__gqa_block_cached__geglu_ffn__decode_kernel(
    A_x: jax.Array,
    A_k_cache: jax.Array,
    A_v_cache: jax.Array,
    A_wq: jax.Array,
    A_wo: jax.Array,
    B_x: jax.Array,
    B_w_gate: jax.Array,
    B_w_up: jax.Array,
    B_w_down: jax.Array,
    grad_out: jax.Array,
):
    del B_x
    _, heads, seq, head_dim = A_k_cache.shape
    d_model = A_x.shape[-1]
    d_ff = B_w_down.shape[0]
    ff_padded = pl.cdiv(d_ff, LANES) * LANES

    args = (
        A_x, A_k_cache, A_v_cache, A_wq, A_wo,
        B_w_gate.T, B_w_up.T, B_w_down, grad_out,
    )
    out_like = (A_x, A_x) + args[1:8]
    hbm = pl.BlockSpec(memory_space=pltpu.HBM)

    out, dx, dk, dv, dwq, dwo, dwg_t, dwu_t, dwd = pl.pallas_call(
        _kernel,
        in_specs=[hbm] * len(args),
        out_specs=[hbm] * len(out_like),
        out_shape=[jax.ShapeDtypeStruct(a.shape, a.dtype) for a in out_like],
        scratch_shapes=[
            pltpu.VMEM((heads, seq, head_dim), BF16),
            pltpu.VMEM((heads, seq, head_dim), BF16),
            pltpu.VMEM(A_wq.shape, BF16),
            pltpu.VMEM(A_wo.shape, BF16),
            pltpu.VMEM((ff_padded, d_model), BF16),
            pltpu.VMEM((ff_padded, d_model), BF16),
            pltpu.VMEM((ff_padded, d_model), BF16),
            pltpu.VMEM(A_x.shape, BF16),
            pltpu.VMEM(A_x.shape, BF16),
            pltpu.VMEM(A_x.shape, BF16),
            pltpu.VMEM(A_x.shape, BF16),
            pltpu.VMEM((ff_padded // LANES, ROWS, LANES), F32),
            pltpu.VMEM((ff_padded // LANES, ROWS, LANES), F32),
            pltpu.VMEM((d_model, LANES), F32),
            pltpu.SemaphoreType.DMA((heads,)),
            pltpu.SemaphoreType.DMA((heads,)),
            pltpu.SemaphoreType.DMA((7,)),
            pltpu.SemaphoreType.DMA((9,)),
        ],
        compiler_params=pltpu.CompilerParams(vmem_limit_bytes=100 * 1024 * 1024),
    )(*args)
    return out, dx, dk, dv, dwq, dwo, dwg_t.T, dwu_t.T, dwd
```

```python
import jax
import jax.numpy as jnp
import jax.experimental.pallas as pl
import jax.experimental.pallas.tpu as pltpu

F32 = jnp.float32
BF16 = jnp.bfloat16
U32 = jnp.uint32
LANES = 128
ROWS = 8
LN_EPS = 1e-5
GELU_C = 0.7978845608028654
GELU_A = 0.044715

READ_BYTES = 64 * 1024
READ_AHEAD = 3
HANDOVER_BLOCKS = 4
DEFERRED_HEADS = 2
WRITE_BYTES = 32 * 1024
WRITE_PLANES = 4
PRIMED_STEPS = 32
TOP_UP_STEPS = 8


def _nn(a, b):
    return jax.lax.dot_general(
        a, b, (((1,), (0,)), ((), ())), preferred_element_type=F32
    )


def _nt(a, b):
    return jax.lax.dot_general(
        a, b, (((1,), (1,)), ((), ())), preferred_element_type=F32
    )


def _column(row):
    return jnp.broadcast_to(row[0:1], (LANES, LANES)).T


def _bf16_rounded(v):
    return v.astype(BF16).astype(F32)


def _gelu_and_grad(z):
    t = jnp.tanh(GELU_C * (z + GELU_A * z * z * z))
    cdf = 0.5 * (1.0 + t)
    pdf = 0.5 * (1.0 - t * t) * GELU_C * (1.0 + 3.0 * GELU_A * z * z)
    return z * cdf, cdf + z * pdf


def _block(j, n):
    return pl.ds(pl.multiple_of(j * n, n), n)


def _loop(lo, hi, body):
    jax.lax.fori_loop(lo, hi, lambda i, _: body(i), None)


def _kernel(
    x_hbm, k_hbm, v_hbm, wq_hbm, wo_hbm, wg_hbm, wu_hbm, wd_hbm, go_hbm,
    out_hbm, dx_hbm, dk_hbm, dv_hbm, dwq_hbm, dwo_hbm, dwg_hbm, dwu_hbm, dwd_hbm,
    k_buf, v_buf, wq_buf, wo_buf, wg_buf, wu_buf, wd_buf,
    x_buf, go_buf, out_buf, dx_buf, gate_buf, up_buf, xcol_buf,
    k_sem, v_sem, sems,
):
    planes, per_plane, seq, head_dim = k_buf.shape
    heads = planes * per_plane
    d_model = wq_buf.shape[0]
    d_attn = heads * head_dim
    d_ff = wg_hbm.shape[0]
    ff_tiles = wg_buf.shape[0] // LANES
    scale = head_dim ** -0.5
    wq_sem, wo_sem, wg_sem, wu_sem, wd_sem, x_sem, go_sem, k_out, v_out = (
        sems.at[i] for i in range(9)
    )

    def copy_rows(src, dst, rows, sem):
        return pltpu.make_async_copy(src.at[rows], dst.at[rows], sem)

    ff_block = READ_BYTES // (2 * d_model)
    ff_full = d_ff // ff_block

    def read_gate_up(j):
        rows = _block(j, ff_block)
        copy_rows(wg_hbm, wg_buf, rows, wg_sem).start(priority=0)
        copy_rows(wu_hbm, wu_buf, rows, wu_sem).start(priority=1)

    def read_down(j):
        for queue in range(2):
            rows = _block(2 * j + queue, ff_block)
            copy_rows(wd_hbm, wd_buf, rows, wd_sem).start(priority=queue)

    def read_attn_weights(j):
        wq_rows = _block(j, READ_BYTES // (2 * d_attn))
        copy_rows(wq_hbm, wq_buf, wq_rows, wq_sem).start(priority=0)
        copy_rows(wo_hbm, wo_buf, _block(j, ff_block), wo_sem).start(priority=1)

    _loop(0, ff_full, read_gate_up)
    x_read = pltpu.make_async_copy(x_hbm, x_buf, x_sem)
    go_read = pltpu.make_async_copy(go_hbm, go_buf, go_sem)
    x_read.start(priority=0)
    go_read.start(priority=1)
    _loop(0, ff_full // 2, read_down)
    for hbm, buf, sem, done, queue in (
        (wg_hbm, wg_buf, wg_sem, ff_full * ff_block, 0),
        (wu_hbm, wu_buf, wu_sem, ff_full * ff_block, 1),
        (wd_hbm, wd_buf, wd_sem, ff_full // 2 * 2 * ff_block, 0),
    ):
        copy_rows(hbm, buf, pl.ds(done, d_ff - done), sem).start(priority=queue)
    _loop(0, d_attn // ff_block, read_attn_weights)

    kv_block = READ_BYTES // (2 * head_dim)
    kv_blocks = seq // kv_block
    kv_slots = k_sem.shape[0] - 1
    last = heads - 1

    def of_head(ref, h):
        return ref.at[h // per_plane, h % per_plane]

    def start_kv(h, slot, lo, hi):
        def body(j):
            rows = _block(j, kv_block)
            copy_rows(
                of_head(k_hbm, h), of_head(k_buf, h), rows, k_sem.at[slot]
            ).start(priority=0)
            copy_rows(
                of_head(v_hbm, h), of_head(v_buf, h), rows, v_sem.at[slot]
            ).start(priority=1)

        _loop(lo, hi, body)

    def wait_kv(h, slot, lo, hi):
        rows = pl.ds(lo * kv_block, (hi - lo) * kv_block)
        copy_rows(of_head(k_hbm, h), of_head(k_buf, h), rows, k_sem.at[slot]).wait()
        copy_rows(of_head(v_hbm, h), of_head(v_buf, h), rows, v_sem.at[slot]).wait()

    x_read.wait()
    go_read.wait()
    x = jnp.broadcast_to(x_buf[0].astype(F32), (ROWS, d_model))
    go = jnp.broadcast_to(go_buf[0].astype(F32), (ROWS, d_model))
    xc = x - jnp.mean(x, axis=-1, keepdims=True)
    rstd = jax.lax.rsqrt(jnp.mean(xc * xc, axis=-1, keepdims=True) + LN_EPS)
    xn = xc * rstd
    xn_b = xn.astype(BF16)
    xn_r = xn_b.astype(F32)
    for t in range(d_model // LANES):
        cols = slice(t * LANES, (t + 1) * LANES)
        xcol_buf[cols, :] = _column(xn_r[:, cols])

    ff_rows = pl.ds(0, d_ff)
    ff_pad = wg_buf.shape[0] - d_ff
    for hbm, buf, sem in (
        (wg_hbm, wg_buf, wg_sem), (wu_hbm, wu_buf, wu_sem), (wd_hbm, wd_buf, wd_sem)
    ):
        copy_rows(hbm, buf, ff_rows, sem).wait()
        buf[pl.ds(d_ff, ff_pad), :] = jnp.zeros((ff_pad, d_model), BF16)
    start_kv(0, 0, 0, kv_blocks)

    def ffn_fwd(t, b):
        rows = _block(t, LANES)
        gate = _nt(xn_b, wg_buf[rows, :])
        up = _nt(xn_b, wu_buf[rows, :])
        gate_buf[t] = gate
        up_buf[t] = up
        act, _ = _gelu_and_grad(gate)
        return b + _nn((act * up).astype(BF16), wd_buf[rows, :])

    zeros = jnp.zeros((ROWS, d_model), F32)
    b = jax.lax.fori_loop(0, ff_tiles, ffn_fwd, zeros)
    sig = jax.nn.sigmoid(b)
    g = b * sig
    ds_b = (go * g).astype(BF16)
    ds_r = ds_b.astype(F32)

    def head(h, s_acc, dxn_acc):
        k_ref, v_ref = of_head(k_buf, h), of_head(v_buf, h)
        span = _block(h, head_dim)
        wq_h = wq_buf[:, span]
        wo_h = wo_buf[span, :]
        q = _nn(xn_b, wq_h)
        do = _nt(ds_b, wo_h)
        scores = _nt(q.astype(BF16), k_ref[...]) * scale
        dp = _nt(do.astype(BF16), v_ref[...])
        e = jnp.exp(scores - jnp.max(scores, axis=-1, keepdims=True))
        p = e * (1.0 / jnp.sum(e, axis=-1, keepdims=True))
        o = _nn(p.astype(BF16), v_ref[...])
        dsc = p * (dp - jnp.sum(p * dp, axis=-1, keepdims=True)) * scale
        dq = _nn(dsc.astype(BF16), k_ref[...])
        s_acc = s_acc + _nn(o.astype(BF16), wo_h)
        dxn_acc = dxn_acc + _nt(dq.astype(BF16), wq_h)

        high = jnp.uint32(0xFFFF0000)
        packed = (pltpu.bitcast(_bf16_rounded(p), U32) & high) | (
            pltpu.bitcast(_bf16_rounded(dsc), U32) >> 16
        )
        do_row = _bf16_rounded(do)[0:1]
        q_row = _bf16_rounded(q)[0:1]
        for t in range(seq // LANES):
            rows = slice(t * LANES, (t + 1) * LANES)
            col = _column(packed[:, rows])
            v_ref[rows, :] = (pltpu.bitcast(col & high, F32) * do_row).astype(BF16)
            k_ref[rows, :] = (pltpu.bitcast(col << 16, F32) * q_row).astype(BF16)

        wq_buf[:, span] = (xcol_buf[...] * _bf16_rounded(dq)[0:1]).astype(BF16)
        o_col = _column(_bf16_rounded(o))
        for t in range(d_model // LANES):
            cols = slice(t * LANES, (t + 1) * LANES)
            wo_buf[span, cols] = (o_col * ds_r[0:1, cols]).astype(BF16)
        return s_acc, dxn_acc

    kv_piece = WRITE_BYTES // (2 * head_dim)
    kv_pieces = seq // kv_piece

    def write_kv(lo, count, also=None):
        def body(i):
            at = (slice(None), i // kv_pieces, _block(i % kv_pieces, kv_piece))
            for j, (buf, hbm, sem) in enumerate(
                ((v_buf, dv_hbm, v_out), (k_buf, dk_hbm, k_out))
            ):
                pltpu.make_async_copy(buf.at[at], hbm.at[at], sem).start()
                if also is not None:
                    also(2 * (i - lo) + j).start()

        _loop(lo, lo + count, body)
        return lo + count

    handover = heads - DEFERRED_HEADS
    cut = kv_blocks - HANDOVER_BLOCKS

    def head_step(h, carry):
        ahead = h + READ_AHEAD

        @pl.when(ahead <= last)
        def _():
            count = jnp.where(ahead == last, cut, kv_blocks)
            start_kv(ahead, ahead % kv_slots, 0, count)

        @pl.when(ahead == last)
        def _():
            start_kv(last, kv_slots, cut, kv_blocks)

        @pl.when(h < handover)
        def _():
            wait_kv(h, h % kv_slots, 0, kv_blocks)

        @pl.when(h == handover)
        def _():
            for t in range(handover, heads):
                wait_kv(t, t % kv_slots, 0, cut if t == last else kv_blocks)
            write_kv(0, PRIMED_STEPS)
            wait_kv(last, kv_slots, cut, kv_blocks)

        @pl.when(h > handover)
        def _():
            write_kv(PRIMED_STEPS + (h - handover - 1) * TOP_UP_STEPS, TOP_UP_STEPS)

        return head(h, *carry)

    _loop(1, READ_AHEAD, lambda h: start_kv(h, h, 0, kv_blocks))
    pltpu.make_async_copy(wq_hbm, wq_buf, wq_sem).wait()
    pltpu.make_async_copy(wo_hbm, wo_buf, wo_sem).wait()
    s, dxn = jax.lax.fori_loop(0, heads, head_step, (zeros, zeros))
    step = write_kv(PRIMED_STEPS + (DEFERRED_HEADS - 1) * TOP_UP_STEPS, TOP_UP_STEPS)

    out_buf[0] = (x + s * g)[0:1].astype(BF16)
    db_b = ((go * s) * (sig * (1.0 + b * (1.0 - sig)))).astype(BF16)
    db_r = db_b.astype(F32)

    def ffn_bwd(t, acc):
        rows = _block(t, LANES)
        up = up_buf[t]
        act, act_grad = _gelu_and_grad(gate_buf[t])
        dh = _nt(db_b, wd_buf[rows, :])
        dgate = (dh * up * act_grad).astype(BF16)
        dup = (dh * act).astype(BF16)
        acc = acc + _nn(dgate, wg_buf[rows, :]) + _nn(dup, wu_buf[rows, :])
        for buf, col_vec, row_vec in (
            (wg_buf, dgate.astype(F32), xn_r),
            (wu_buf, dup.astype(F32), xn_r),
            (wd_buf, _bf16_rounded(act * up), db_r),
        ):
            col = _column(col_vec)
            for c in range(d_model // LANES):
                cols = slice(c * LANES, (c + 1) * LANES)
                buf[rows, cols] = (col * row_vec[0:1, cols]).astype(BF16)
        return acc

    dxn = jax.lax.fori_loop(0, ff_tiles, ffn_bwd, dxn)
    dx = go + rstd * (
        dxn
        - jnp.mean(dxn, axis=-1, keepdims=True)
        - xn * jnp.mean(dxn * xn, axis=-1, keepdims=True)
    )
    dx_buf[0] = dx[0:1].astype(BF16)

    out_write = pltpu.make_async_copy(out_buf, out_hbm, x_sem)
    dx_write = pltpu.make_async_copy(dx_buf, dx_hbm, go_sem)
    out_write.start()
    dx_write.start()

    piece = WRITE_BYTES // (2 * d_model)
    wq_width = WRITE_BYTES // (2 * 8)
    wq_splits = d_attn // wq_width

    def wq_write(j):
        at = (_block(j // wq_splits, 8), _block(j % wq_splits, wq_width))
        return pltpu.make_async_copy(wq_buf.at[at], dwq_hbm.at[at], wq_sem)

    def row_write(buf, hbm, sem):
        return lambda j: copy_rows(buf, hbm, _block(j, piece), sem)

    ffn_outputs = (
        (wg_buf, dwg_hbm, wg_sem), (wu_buf, dwu_hbm, wu_sem), (wd_buf, dwd_hbm, wd_sem)
    )
    step = write_kv(step, d_attn // piece // 2, wq_write)
    step = write_kv(step, d_attn // piece // 2, row_write(wo_buf, dwo_hbm, wo_sem))
    for buf, hbm, sem in ffn_outputs:
        pairs = d_ff // piece // 2
        step = write_kv(step, pairs, row_write(buf, hbm, sem))
        done = 2 * pairs * piece
        copy_rows(buf, hbm, pl.ds(done, d_ff - done), sem).start()
    write_kv(step, per_plane * kv_pieces - step)

    out_write.wait()
    dx_write.wait()
    pltpu.make_async_copy(wq_buf, dwq_hbm, wq_sem).wait()
    pltpu.make_async_copy(wo_buf, dwo_hbm, wo_sem).wait()
    for buf, hbm, sem in ffn_outputs:
        copy_rows(buf, hbm, ff_rows, sem).wait()
    pltpu.make_async_copy(v_buf, dv_hbm, v_out).wait()
    pltpu.make_async_copy(k_buf, dk_hbm, k_out).wait()


@jax.jit
def pallas_recurrent_scan__gqa_block_cached__geglu_ffn__decode_kernel(
    A_x: jax.Array,
    A_k_cache: jax.Array,
    A_v_cache: jax.Array,
    A_wq: jax.Array,
    A_wo: jax.Array,
    B_x: jax.Array,
    B_w_gate: jax.Array,
    B_w_up: jax.Array,
    B_w_down: jax.Array,
    grad_out: jax.Array,
):
    del B_x
    _, heads, seq, head_dim = A_k_cache.shape
    d_model = A_x.shape[-1]
    d_ff = B_w_down.shape[0]
    ff_padded = pl.cdiv(d_ff, LANES) * LANES
    cache = (WRITE_PLANES, heads // WRITE_PLANES, seq, head_dim)

    args = (
        A_x, A_k_cache.reshape(cache), A_v_cache.reshape(cache), A_wq, A_wo,
        B_w_gate.T, B_w_up.T, B_w_down, grad_out,
    )
    out_like = (A_x, A_x) + args[1:8]
    hbm = pl.BlockSpec(memory_space=pltpu.HBM)

    out, dx, dk, dv, dwq, dwo, dwg_t, dwu_t, dwd = pl.pallas_call(
        _kernel,
        in_specs=[hbm] * len(args),
        out_specs=[hbm] * len(out_like),
        out_shape=[jax.ShapeDtypeStruct(a.shape, a.dtype) for a in out_like],
        scratch_shapes=[
            pltpu.VMEM(cache, BF16),
            pltpu.VMEM(cache, BF16),
            pltpu.VMEM(A_wq.shape, BF16),
            pltpu.VMEM(A_wo.shape, BF16),
            pltpu.VMEM((ff_padded, d_model), BF16),
            pltpu.VMEM((ff_padded, d_model), BF16),
            pltpu.VMEM((ff_padded, d_model), BF16),
            pltpu.VMEM(A_x.shape, BF16),
            pltpu.VMEM(A_x.shape, BF16),
            pltpu.VMEM(A_x.shape, BF16),
            pltpu.VMEM(A_x.shape, BF16),
            pltpu.VMEM((ff_padded // LANES, ROWS, LANES), F32),
            pltpu.VMEM((ff_padded // LANES, ROWS, LANES), F32),
            pltpu.VMEM((d_model, LANES), F32),
            pltpu.SemaphoreType.DMA((READ_AHEAD + 2,)),
            pltpu.SemaphoreType.DMA((READ_AHEAD + 2,)),
            pltpu.SemaphoreType.DMA((9,)),
        ],
        compiler_params=pltpu.CompilerParams(vmem_limit_bytes=100 * 1024 * 1024),
    )(*args)
    return (
        out, dx, dk.reshape(A_k_cache.shape), dv.reshape(A_v_cache.shape),
        dwq, dwo, dwg_t.T, dwu_t.T, dwd,
    )
```

```python
import jax
import jax.numpy as jnp
import jax.experimental.pallas as pl
import jax.experimental.pallas.tpu as pltpu

F32 = jnp.float32
BF16 = jnp.bfloat16
U32 = jnp.uint32
LANES = 128
ROWS = 8
LN_EPS = 1e-5
GELU_C = 0.7978845608028654
GELU_A = 0.044715

ATTN_PLANES = 4
FFN_PLANES = 2
ATTN_READ_ROWS = 8
ATTN_WRITE_ROWS = 16
FFN_ROWS = 16

READ_HEADS = 8
READ_ROWS = 16
COMPUTE_LAG = READ_HEADS + 1
HANDOVER_READS = 16

WRITE_GROUPS = (7, 7, 6, 6, 6)
WRITE_ROWS = 64
PRIMED_WRITES = 64
TOP_UP_WRITES = 13


def _nn(a, b):
    return jax.lax.dot_general(
        a, b, (((1,), (0,)), ((), ())), preferred_element_type=F32
    )


def _nt(a, b):
    return jax.lax.dot_general(
        a, b, (((1,), (1,)), ((), ())), preferred_element_type=F32
    )


def _column(row):
    return jnp.broadcast_to(row[0:1], (LANES, LANES)).T


def _bf16_rounded(v):
    return v.astype(BF16).astype(F32)


def _gelu_and_grad(z):
    t = jnp.tanh(GELU_C * (z + GELU_A * z * z * z))
    cdf = 0.5 * (1.0 + t)
    pdf = 0.5 * (1.0 - t * t) * GELU_C * (1.0 + 3.0 * GELU_A * z * z)
    return z * cdf, cdf + z * pdf


def _block(j, n):
    return pl.ds(pl.multiple_of(j * n, n), n)


def _loop(lo, hi, body):
    def step(i, carry):
        body(i)
        return carry

    jax.lax.fori_loop(lo, hi, step, None)


def _copy(src, dst, at, sem):
    return pltpu.make_async_copy(src.at[at], dst.at[at], sem)


def _kernel(
    x_hbm, k_hbm, v_hbm, wq_hbm, wo_hbm, wg_hbm, wu_hbm, wd_hbm, go_hbm,
    out_hbm, dx_hbm, dk_hbm, dv_hbm, dwq_hbm, dwo_hbm, dwg_hbm, dwu_hbm, dwd_hbm,
    k_buf, v_buf, wq_buf, wo_buf, wg_buf, wu_buf, wd_buf,
    x_buf, go_buf, out_buf, dx_buf, gate_buf, up_buf, xcol_buf,
    k_sem, v_sem, sems,
):
    heads, seq, head_dim = k_buf.shape
    d_model = x_buf.shape[-1]
    d_attn = heads * head_dim
    heads_per_plane = heads // ATTN_PLANES
    wo_rows = wo_buf.shape[1]
    ff_rows = wg_hbm.shape[1]
    ff_tiles = wg_buf.shape[1] // LANES
    scale = head_dim ** -0.5
    all_planes = slice(None)
    wq_sem, wo_sem, wg_sem, wu_sem, wd_sem, x_sem, go_sem, dk_sem, dv_sem = (
        sems.at[i] for i in range(9)
    )
    ffn = (
        (wg_hbm, wg_buf, dwg_hbm, wg_sem),
        (wu_hbm, wu_buf, dwu_hbm, wu_sem),
        (wd_hbm, wd_buf, dwd_hbm, wd_sem),
    )

    def wq_piece(j, wo_piece_rows):
        width = wo_piece_rows * d_model // 8
        per_row = d_attn // width
        return (all_planes, _block(j // per_row, 8), _block(j % per_row, width))

    def read_attn_weights(j):
        _copy(wq_hbm, wq_buf, wq_piece(j, ATTN_READ_ROWS), wq_sem).start(priority=0)
        at = (all_planes, _block(j, ATTN_READ_ROWS))
        _copy(wo_hbm, wo_buf, at, wo_sem).start(priority=1)

    def read_ffn_weights(j, parity):
        for i, (hbm, buf, _, sem) in enumerate(ffn):
            at = (all_planes, _block(j, FFN_ROWS))
            _copy(hbm, buf, at, sem).start(priority=(i + parity) % 2)

    def read_ffn_pair(j):
        read_ffn_weights(2 * j, 0)
        read_ffn_weights(2 * j + 1, 1)

    x_read = pltpu.make_async_copy(x_hbm, x_buf, x_sem)
    go_read = pltpu.make_async_copy(go_hbm, go_buf, go_sem)
    ffn_pieces = ff_rows // FFN_ROWS
    _loop(0, wo_rows // ATTN_READ_ROWS, read_attn_weights)
    x_read.start(priority=0)
    go_read.start(priority=1)
    _loop(0, ffn_pieces // 2, read_ffn_pair)
    if ffn_pieces % 2:
        read_ffn_weights(ffn_pieces - 1, 0)

    reads_per_step = seq // READ_HEADS // READ_ROWS
    last_group = heads // READ_HEADS - 1

    def start_reads(t, slot, lo, hi):
        def body(j):
            piece = (t % READ_HEADS) * reads_per_step + j
            at = (_block(t // READ_HEADS, READ_HEADS), _block(piece, READ_ROWS))
            _copy(k_hbm, k_buf, at, k_sem.at[slot]).start(priority=0)
            _copy(v_hbm, v_buf, at, v_sem.at[slot]).start(priority=1)

        _loop(lo, hi, body)

    def read_step(t):
        start_reads(t, t // READ_HEADS, 0, reads_per_step)

    def wait_reads(group, slot, lo, hi):
        at = (_block(group, READ_HEADS), pl.ds(lo, hi - lo))
        _copy(k_hbm, k_buf, at, k_sem.at[slot]).wait()
        _copy(v_hbm, v_buf, at, v_sem.at[slot]).wait()

    x_read.wait()
    go_read.wait()
    read_step(0)
    x = jnp.broadcast_to(x_buf[0].astype(F32), (ROWS, d_model))
    go = jnp.broadcast_to(go_buf[0].astype(F32), (ROWS, d_model))
    xc = x - jnp.mean(x, axis=-1, keepdims=True)
    rstd = jax.lax.rsqrt(jnp.mean(xc * xc, axis=-1, keepdims=True) + LN_EPS)
    xn = xc * rstd
    xn_b = xn.astype(BF16)
    xn_r = xn_b.astype(F32)
    for t in range(d_model // LANES):
        cols = slice(t * LANES, (t + 1) * LANES)
        xcol_buf[cols, :] = _column(xn_r[:, cols])

    _loop(1, 3, read_step)
    ff_data = (all_planes, pl.ds(0, ff_rows))
    ff_pad = wg_buf.shape[1] - ff_rows
    for hbm, buf, _, sem in ffn:
        _copy(hbm, buf, ff_data, sem).wait()
        buf[:, pl.ds(ff_rows, ff_pad), :] = jnp.zeros(
            (FFN_PLANES, ff_pad, d_model), BF16
        )

    def ffn_tile(t):
        return (t // ff_tiles, _block(t % ff_tiles, LANES))

    def ffn_fwd(t, b):
        at = ffn_tile(t)
        gate = _nt(xn_b, wg_buf[at])
        up = _nt(xn_b, wu_buf[at])
        gate_buf[t] = gate
        up_buf[t] = up
        act, _ = _gelu_and_grad(gate)
        return b + _nn((act * up).astype(BF16), wd_buf[at])

    zeros = jnp.zeros((ROWS, d_model), F32)
    b = jax.lax.fori_loop(0, FFN_PLANES * ff_tiles, ffn_fwd, zeros)
    sig = jax.nn.sigmoid(b)
    g = b * sig
    ds_b = (go * g).astype(BF16)
    ds_r = ds_b.astype(F32)

    def head(h, s_acc, dxn_acc):
        k_ref, v_ref = k_buf.at[h], v_buf.at[h]
        wo_ref = wo_buf.at[h // heads_per_plane, _block(h % heads_per_plane, head_dim)]
        span = _block(h, head_dim)
        wq_h = wq_buf[:, :, span].reshape(d_model, head_dim)
        wo_h = wo_ref[...]
        q = _nn(xn_b, wq_h)
        do = _nt(ds_b, wo_h)
        scores = _nt(q.astype(BF16), k_ref[...]) * scale
        dp = _nt(do.astype(BF16), v_ref[...])
        e = jnp.exp(scores - jnp.max(scores, axis=-1, keepdims=True))
        p = e * (1.0 / jnp.sum(e, axis=-1, keepdims=True))
        o = _nn(p.astype(BF16), v_ref[...])
        dsc = p * (dp - jnp.sum(p * dp, axis=-1, keepdims=True)) * scale
        dq = _nn(dsc.astype(BF16), k_ref[...])
        s_acc = s_acc + _nn(o.astype(BF16), wo_h)
        dxn_acc = dxn_acc + _nt(dq.astype(BF16), wq_h)

        high = jnp.uint32(0xFFFF0000)
        packed = (pltpu.bitcast(_bf16_rounded(p), U32) & high) | (
            pltpu.bitcast(_bf16_rounded(dsc), U32) >> 16
        )
        do_row = _bf16_rounded(do)[0:1]
        q_row = _bf16_rounded(q)[0:1]
        for t in range(seq // LANES):
            rows = slice(t * LANES, (t + 1) * LANES)
            col = _column(packed[:, rows])
            v_ref[rows, :] = (pltpu.bitcast(col & high, F32) * do_row).astype(BF16)
            k_ref[rows, :] = (pltpu.bitcast(col << 16, F32) * q_row).astype(BF16)

        dwq_h = (xcol_buf[...] * _bf16_rounded(dq)[0:1]).astype(BF16)
        wq_buf[:, :, span] = dwq_h.reshape(ATTN_PLANES, -1, head_dim)
        o_col = _column(_bf16_rounded(o))
        for t in range(d_model // LANES):
            cols = slice(t * LANES, (t + 1) * LANES)
            wo_ref[:, cols] = (o_col * ds_r[0:1, cols]).astype(BF16)
        return s_acc, dxn_acc

    writes_per_cache = seq // WRITE_ROWS

    def write_caches(size, first_head, lo, count):
        def body(j):
            i = lo + j
            run = i // writes_per_cache
            at = (
                pl.ds(first_head + run // 2 * size, size),
                _block(i % writes_per_cache, WRITE_ROWS),
            )
            pl.when(run % 2 == 0)(lambda: _copy(v_buf, dv_hbm, at, dv_sem).start())
            pl.when(run % 2 == 1)(lambda: _copy(k_buf, dk_hbm, at, dk_sem).start())

        _loop(0, count, body)

    early_size = WRITE_GROUPS[0]
    assert WRITE_GROUPS[1] == early_size and 2 * early_size <= heads - COMPUTE_LAG

    def step(t, carry):
        h = t - COMPUTE_LAG
        pl.when(t < heads - 1)(lambda: read_step(t))

        @pl.when(t == heads - 1)
        def _():
            cut = reads_per_step - HANDOVER_READS
            start_reads(heads - 1, last_group, 0, cut)
            start_reads(heads - 1, last_group + 1, cut, reads_per_step)

        @pl.when((h % READ_HEADS == 0) & (h // READ_HEADS < last_group))
        def _():
            wait_reads(h // READ_HEADS, h // READ_HEADS, 0, seq)

        @pl.when(t == heads)
        def _():
            split = seq - HANDOVER_READS * READ_ROWS
            wait_reads(last_group, last_group, 0, split)
            write_caches(early_size, 0, 0, PRIMED_WRITES)
            wait_reads(last_group, last_group + 1, split, seq)

        @pl.when(t > heads)
        def _():
            lo = PRIMED_WRITES + (t - heads - 1) * TOP_UP_WRITES
            write_caches(early_size, 0, lo, TOP_UP_WRITES)

        return head(h, *carry)

    _loop(3, COMPUTE_LAG, read_step)
    pltpu.make_async_copy(wq_hbm, wq_buf, wq_sem).wait()
    pltpu.make_async_copy(wo_hbm, wo_buf, wo_sem).wait()
    s, dxn = jax.lax.fori_loop(COMPUTE_LAG, heads + COMPUTE_LAG, step, (zeros, zeros))
    written = PRIMED_WRITES + (COMPUTE_LAG - 1) * TOP_UP_WRITES
    write_caches(early_size, 0, written, 2 * TOP_UP_WRITES)
    written += 2 * TOP_UP_WRITES

    out_buf[0] = (x + s * g)[0:1].astype(BF16)
    db_b = ((go * s) * (sig * (1.0 + b * (1.0 - sig)))).astype(BF16)
    db_r = db_b.astype(F32)

    def ffn_bwd(t, acc):
        at = ffn_tile(t)
        up = up_buf[t]
        act, act_grad = _gelu_and_grad(gate_buf[t])
        dh = _nt(db_b, wd_buf[at])
        dgate = (dh * up * act_grad).astype(BF16)
        dup = (dh * act).astype(BF16)
        acc = acc + _nn(dgate, wg_buf[at]) + _nn(dup, wu_buf[at])
        for buf, col_vec, row_vec in (
            (wg_buf, dgate.astype(F32), xn_r),
            (wu_buf, dup.astype(F32), xn_r),
            (wd_buf, _bf16_rounded(act * up), db_r),
        ):
            col = _column(col_vec)
            for c in range(d_model // LANES):
                cols = slice(c * LANES, (c + 1) * LANES)
                buf[at + (cols,)] = (col * row_vec[0:1, cols]).astype(BF16)
        return acc

    dxn = jax.lax.fori_loop(0, FFN_PLANES * ff_tiles, ffn_bwd, dxn)
    dx = go + rstd * (
        dxn
        - jnp.mean(dxn, axis=-1, keepdims=True)
        - xn * jnp.mean(dxn * xn, axis=-1, keepdims=True)
    )
    dx_buf[0] = dx[0:1].astype(BF16)

    def write_attn_weights(j):
        _copy(wq_buf, dwq_hbm, wq_piece(j, ATTN_WRITE_ROWS), wq_sem).start()
        at = (all_planes, _block(j, ATTN_WRITE_ROWS))
        _copy(wo_buf, dwo_hbm, at, wo_sem).start()

    def write_ffn_weights(j):
        for _, buf, hbm, sem in ffn:
            _copy(buf, hbm, (all_planes, _block(j, FFN_ROWS)), sem).start()

    out_write = pltpu.make_async_copy(out_buf, out_hbm, x_sem)
    dx_write = pltpu.make_async_copy(dx_buf, dx_hbm, go_sem)
    out_write.start()
    dx_write.start()
    write_caches(early_size, 0, written, 4 * writes_per_cache - written)
    _loop(0, wo_rows // ATTN_WRITE_ROWS, write_attn_weights)
    _loop(0, ffn_pieces, write_ffn_weights)
    first_head = 2 * early_size
    for size in WRITE_GROUPS[2:]:
        write_caches(size, first_head, 0, 2 * writes_per_cache)
        first_head += size

    out_write.wait()
    dx_write.wait()
    pltpu.make_async_copy(wq_buf, dwq_hbm, wq_sem).wait()
    pltpu.make_async_copy(wo_buf, dwo_hbm, wo_sem).wait()
    for _, buf, hbm, sem in ffn:
        _copy(buf, hbm, ff_data, sem).wait()
    pltpu.make_async_copy(v_buf, dv_hbm, dv_sem).wait()
    pltpu.make_async_copy(k_buf, dk_hbm, dk_sem).wait()


@jax.jit
def pallas_recurrent_scan__gqa_block_cached__geglu_ffn__decode_kernel(
    A_x: jax.Array,
    A_k_cache: jax.Array,
    A_v_cache: jax.Array,
    A_wq: jax.Array,
    A_wo: jax.Array,
    B_x: jax.Array,
    B_w_gate: jax.Array,
    B_w_up: jax.Array,
    B_w_down: jax.Array,
    grad_out: jax.Array,
):
    del B_x
    _, heads, seq, head_dim = A_k_cache.shape
    d_model = A_x.shape[-1]
    d_attn = heads * head_dim
    d_ff = B_w_down.shape[0]
    cache = (heads, seq, head_dim)
    ff = (FFN_PLANES, d_ff // FFN_PLANES, d_model)
    ff_padded = (FFN_PLANES, pl.cdiv(ff[1], LANES) * LANES, d_model)
    ff_tiles = FFN_PLANES * ff_padded[1] // LANES
    assert heads == sum(WRITE_GROUPS) and ff[1] % FFN_ROWS == 0

    args = (
        A_x,
        A_k_cache.reshape(cache),
        A_v_cache.reshape(cache),
        A_wq.reshape(ATTN_PLANES, d_model // ATTN_PLANES, d_attn),
        A_wo.reshape(ATTN_PLANES, d_attn // ATTN_PLANES, d_model),
        B_w_gate.T.reshape(ff),
        B_w_up.T.reshape(ff),
        B_w_down.reshape(ff),
        grad_out,
    )
    out_like = (A_x, A_x) + args[1:8]
    hbm = pl.BlockSpec(memory_space=pltpu.HBM)

    out, dx, dk, dv, dwq, dwo, dwg_t, dwu_t, dwd = pl.pallas_call(
        _kernel,
        in_specs=[hbm] * len(args),
        out_specs=[hbm] * len(out_like),
        out_shape=[jax.ShapeDtypeStruct(a.shape, a.dtype) for a in out_like],
        scratch_shapes=[
            *(pltpu.VMEM(a.shape, BF16) for a in args[1:5]),
            *[pltpu.VMEM(ff_padded, BF16)] * 3,
            *[pltpu.VMEM(A_x.shape, BF16)] * 4,
            *[pltpu.VMEM((ff_tiles, ROWS, LANES), F32)] * 2,
            pltpu.VMEM((d_model, LANES), F32),
            *[pltpu.SemaphoreType.DMA((heads // READ_HEADS + 1,))] * 2,
            pltpu.SemaphoreType.DMA((9,)),
        ],
        compiler_params=pltpu.CompilerParams(
            vmem_limit_bytes=100 * 1024 * 1024,
            disable_bounds_checks=True,
            disable_semaphore_checks=True,
        ),
    )(*args)
    return (
        out,
        dx,
        dk.reshape(A_k_cache.shape),
        dv.reshape(A_v_cache.shape),
        dwq.reshape(A_wq.shape),
        dwo.reshape(A_wo.shape),
        dwg_t.reshape(d_ff, d_model).T,
        dwu_t.reshape(d_ff, d_model).T,
        dwd.reshape(d_ff, d_model),
    )
```

```python
import jax
import jax.numpy as jnp
import jax.experimental.pallas as pl
import jax.experimental.pallas.tpu as pltpu

F32 = jnp.float32
BF16 = jnp.bfloat16
U32 = jnp.uint32
LANES = 128
ROWS = 8
LN_EPS = 1e-5
GELU_C = 0.7978845608028654
GELU_A = 0.044715

ATTN_PLANES = 4
FFN_PLANES = 2
ATTN_READ_ROWS = 8
ATTN_WRITE_ROWS = 16
FFN_ROWS = 16

READ_HEADS = 8
READ_ROWS = 16
COMPUTE_LAG = READ_HEADS + 1
HANDOVER_READS = 14

WRITE_GROUPS = ((6, 3), (7, 2))
WRITE_ROWS = 64
WRITES_AT_HANDOVER = 64
WRITES_PER_ATTENTION_HEAD = 16
WRITES_PER_PROJECTION_HEAD = 3
WRITES_PER_FFN_TILE = 8


def _nn(a, b):
    return jax.lax.dot_general(
        a, b, (((1,), (0,)), ((), ())), preferred_element_type=F32
    )


def _nt(a, b):
    return jax.lax.dot_general(
        a, b, (((1,), (1,)), ((), ())), preferred_element_type=F32
    )


def _column(row):
    return jnp.broadcast_to(row[0:1], (LANES, LANES)).T


def _bf16_rounded(v):
    return v.astype(BF16).astype(F32)


def _gelu_and_grad(z):
    t = jnp.tanh(GELU_C * (z + GELU_A * z * z * z))
    cdf = 0.5 * (1.0 + t)
    pdf = 0.5 * (1.0 - t * t) * GELU_C * (1.0 + 3.0 * GELU_A * z * z)
    return z * cdf, cdf + z * pdf


def _block(j, n):
    return pl.ds(pl.multiple_of(j * n, n), n)


def _loop(lo, hi, body, unroll=1):
    assert (hi - lo) % unroll == 0

    def step(i, carry):
        for u in range(unroll):
            body(lo + i * unroll + u)
        return carry

    jax.lax.fori_loop(0, (hi - lo) // unroll, step, None)


def _copy(src, dst, at, sem):
    return pltpu.make_async_copy(src.at[at], dst.at[at], sem)


def _kernel(
    x_hbm, k_hbm, v_hbm, wq_hbm, wo_hbm, wg_hbm, wu_hbm, wd_hbm, go_hbm,
    out_hbm, dx_hbm, dk_hbm, dv_hbm, dwq_hbm, dwo_hbm, dwg_hbm, dwu_hbm, dwd_hbm,
    k_buf, v_buf, wq_buf, wo_buf, wg_buf, wu_buf, wd_buf,
    x_buf, go_buf, out_buf, dx_buf, gate_buf, up_buf, q_buf, o_buf, xcol_buf,
    k_sem, v_sem, sems,
):
    heads, seq, head_dim = k_buf.shape
    d_model = x_buf.shape[-1]
    d_attn = heads * head_dim
    heads_per_plane = heads // ATTN_PLANES
    wo_rows = wo_buf.shape[1]
    ff_rows = wg_hbm.shape[1]
    tiles_per_plane = wg_buf.shape[1] // LANES
    ff_tiles = FFN_PLANES * tiles_per_plane
    scale = head_dim ** -0.5
    all_planes = slice(None)
    wq_sem, wo_sem, wg_sem, wu_sem, wd_sem, x_sem, go_sem, dk_sem, dv_sem = (
        sems.at[i] for i in range(9)
    )
    ffn = (
        (wg_hbm, wg_buf, dwg_hbm, wg_sem),
        (wu_hbm, wu_buf, dwu_hbm, wu_sem),
        (wd_hbm, wd_buf, dwd_hbm, wd_sem),
    )

    def wq_piece(j, wo_piece_rows):
        width = wo_piece_rows * d_model // 8
        per_row = d_attn // width
        return (all_planes, _block(j // per_row, 8), _block(j % per_row, width))

    def read_attn_weights(j):
        _copy(wq_hbm, wq_buf, wq_piece(j, ATTN_READ_ROWS), wq_sem).start(priority=0)
        at = (all_planes, _block(j, ATTN_READ_ROWS))
        _copy(wo_hbm, wo_buf, at, wo_sem).start(priority=1)

    def read_ffn_weights(j, parity):
        for i, (hbm, buf, _, sem) in enumerate(ffn):
            at = (all_planes, _block(j, FFN_ROWS))
            _copy(hbm, buf, at, sem).start(priority=(i + parity) % 2)

    def read_ffn_pair(j):
        read_ffn_weights(2 * j, 0)
        read_ffn_weights(2 * j + 1, 1)

    x_read = pltpu.make_async_copy(x_hbm, x_buf, x_sem)
    go_read = pltpu.make_async_copy(go_hbm, go_buf, go_sem)
    ffn_pieces = ff_rows // FFN_ROWS
    read_attn_weights(0)
    _loop(1, wo_rows // ATTN_READ_ROWS, read_attn_weights)
    x_read.start(priority=0)
    go_read.start(priority=1)
    _loop(0, ffn_pieces // 2, read_ffn_pair)
    if ffn_pieces % 2:
        read_ffn_weights(ffn_pieces - 1, 0)

    reads_per_step = seq // READ_HEADS // READ_ROWS
    last_group = heads // READ_HEADS - 1

    def start_reads(t, slot, lo, hi, unroll=1):
        def body(j):
            piece = (t % READ_HEADS) * reads_per_step + j
            at = (_block(t // READ_HEADS, READ_HEADS), _block(piece, READ_ROWS))
            _copy(k_hbm, k_buf, at, k_sem.at[slot]).start(priority=0)
            _copy(v_hbm, v_buf, at, v_sem.at[slot]).start(priority=1)

        _loop(lo, hi, body, unroll)

    def read_step(t, unroll=1):
        start_reads(t, t // READ_HEADS, 0, reads_per_step, unroll)

    def wait_reads(group, slot, lo, hi):
        at = (_block(group, READ_HEADS), pl.ds(lo, hi - lo))
        _copy(k_hbm, k_buf, at, k_sem.at[slot]).wait()
        _copy(v_hbm, v_buf, at, v_sem.at[slot]).wait()

    x_read.wait()
    go_read.wait()
    read_step(0)
    x = jnp.broadcast_to(x_buf[0].astype(F32), (ROWS, d_model))
    go = jnp.broadcast_to(go_buf[0].astype(F32), (ROWS, d_model))
    xc = x - jnp.mean(x, axis=-1, keepdims=True)
    rstd = jax.lax.rsqrt(jnp.mean(xc * xc, axis=-1, keepdims=True) + LN_EPS)
    xn = xc * rstd
    xn_b = xn.astype(BF16)
    xn_r = xn_b.astype(F32)
    for t in range(d_model // LANES):
        cols = slice(t * LANES, (t + 1) * LANES)
        xcol_buf[cols, :] = _column(xn_r[:, cols])

    _loop(1, 3, read_step)
    ff_data = (all_planes, pl.ds(0, ff_rows))
    ff_pad = wg_buf.shape[1] - ff_rows
    for hbm, buf, _, sem in ffn:
        _copy(hbm, buf, ff_data, sem).wait()
        buf[:, pl.ds(ff_rows, ff_pad), :] = jnp.zeros(
            (FFN_PLANES, ff_pad, d_model), BF16
        )

    def ffn_tile(t):
        return (t // tiles_per_plane, _block(t % tiles_per_plane, LANES))

    def ffn_fwd(t, b):
        pl.when(t % 4 == 1)(lambda: read_step(3 + t // 4))
        at = ffn_tile(t)
        gate = _nt(xn_b, wg_buf[at])
        up = _nt(xn_b, wu_buf[at])
        gate_buf[t] = gate
        up_buf[t] = up
        act, _ = _gelu_and_grad(gate)
        return b + _nn((act * up).astype(BF16), wd_buf[at])

    zeros = jnp.zeros((ROWS, d_model), F32)
    b = jax.lax.fori_loop(0, ff_tiles, ffn_fwd, zeros)
    sig = jax.nn.sigmoid(b)
    g = b * sig
    ds_b = (go * g).astype(BF16)
    ds_r = ds_b.astype(F32)

    def wq_columns(cols):
        return wq_buf[:, :, cols].reshape(d_model, -1)

    def project_in(plane):
        cols = _block(plane, wo_rows)
        q_buf[:, cols] = _bf16_rounded(_nn(xn_b, wq_columns(cols)))
        o_buf[:, cols] = _bf16_rounded(_nt(ds_b, wo_buf[plane]))

    pltpu.make_async_copy(wq_hbm, wq_buf, wq_sem).wait()
    pltpu.make_async_copy(wo_hbm, wo_buf, wo_sem).wait()
    steps_read = 3 + (ff_tiles + 2) // 4
    read_step(steps_read)
    _loop(0, ATTN_PLANES, project_in)
    _loop(steps_read + 1, COMPUTE_LAG, read_step)

    def attend(h):
        k_ref, v_ref = k_buf.at[h], v_buf.at[h]
        span = _block(h, head_dim)
        q = q_buf[:, span]
        do = o_buf[:, span]
        scores = _nt(q.astype(BF16), k_ref[...]) * scale
        dp = _nt(do.astype(BF16), v_ref[...])
        e = jnp.exp(scores - jnp.max(scores, axis=-1, keepdims=True))
        p = e * (1.0 / jnp.sum(e, axis=-1, keepdims=True))
        dsc = p * (dp - jnp.sum(p * dp, axis=-1, keepdims=True)) * scale
        o_buf[:, span] = _nn(p.astype(BF16), v_ref[...])
        q_buf[:, span] = _nn(dsc.astype(BF16), k_ref[...])

        high = jnp.uint32(0xFFFF0000)
        packed = (pltpu.bitcast(_bf16_rounded(p), U32) & high) | (
            pltpu.bitcast(_bf16_rounded(dsc), U32) >> 16
        )
        for t in range(seq // LANES):
            rows = slice(t * LANES, (t + 1) * LANES)
            col = _column(packed[:, rows])
            v_ref[rows, :] = (pltpu.bitcast(col & high, F32) * do[0:1]).astype(BF16)
            k_ref[rows, :] = (pltpu.bitcast(col << 16, F32) * q[0:1]).astype(BF16)

    writes_per_cache = seq // WRITE_ROWS

    def write_caches(size, first_head, lo, count):
        def body(j):
            i = lo + j
            run = i // writes_per_cache
            at = (
                pl.ds(first_head + run // 2 * size, size),
                _block(i % writes_per_cache, WRITE_ROWS),
            )
            pl.when(run % 2 == 0)(lambda: _copy(v_buf, dv_hbm, at, dv_sem).start())
            pl.when(run % 2 == 1)(lambda: _copy(k_buf, dk_hbm, at, dk_sem).start())

        _loop(0, count, body)

    early_size, early_groups = WRITE_GROUPS[0]
    assert early_size * early_groups <= heads - COMPUTE_LAG

    def write_early(lo, count):
        write_caches(early_size, 0, lo, count)

    def step(t):
        h = t - COMPUTE_LAG
        pl.when(t < heads - 1)(lambda: read_step(t, unroll=8))

        @pl.when(t == heads - 1)
        def _():
            cut = reads_per_step - HANDOVER_READS
            start_reads(heads - 1, last_group, 0, cut)
            start_reads(heads - 1, last_group + 1, cut, reads_per_step)

        @pl.when((h % READ_HEADS == 0) & (h // READ_HEADS < last_group))
        def _():
            wait_reads(h // READ_HEADS, h // READ_HEADS, 0, seq)

        @pl.when(t == heads)
        def _():
            split = seq - HANDOVER_READS * READ_ROWS
            wait_reads(last_group, last_group, 0, split)
            write_early(0, WRITES_AT_HANDOVER)
            wait_reads(last_group, last_group + 1, split, seq)

        @pl.when(t > heads)
        def _():
            done = (t - heads - 1) * WRITES_PER_ATTENTION_HEAD
            write_early(WRITES_AT_HANDOVER + done, WRITES_PER_ATTENTION_HEAD)

        attend(h)

    _loop(COMPUTE_LAG, heads + COMPUTE_LAG, step)
    attention_writes = (
        WRITES_AT_HANDOVER + (COMPUTE_LAG - 1) * WRITES_PER_ATTENTION_HEAD
    )

    def project_out(h, carry):
        s_acc, dxn_acc = carry
        done = h * WRITES_PER_PROJECTION_HEAD
        write_early(attention_writes + done, WRITES_PER_PROJECTION_HEAD)
        wo_ref = wo_buf.at[h // heads_per_plane, _block(h % heads_per_plane, head_dim)]
        span = _block(h, head_dim)
        o = o_buf[:, span].astype(BF16)
        dq = q_buf[:, span].astype(BF16)
        s_acc = s_acc + _nn(o, wo_ref[...])
        dxn_acc = dxn_acc + _nt(dq, wq_columns(span))
        dwq = (xcol_buf[...] * dq.astype(F32)[0:1]).astype(BF16)
        wq_buf[:, :, span] = dwq.reshape(ATTN_PLANES, -1, head_dim)
        o_col = _column(o.astype(F32))
        for c in range(d_model // LANES):
            cols = slice(c * LANES, (c + 1) * LANES)
            wo_ref[:, cols] = (o_col * ds_r[0:1, cols]).astype(BF16)
        return s_acc, dxn_acc

    s, dxn = jax.lax.fori_loop(0, heads, project_out, (zeros, zeros))
    projection_writes = attention_writes + heads * WRITES_PER_PROJECTION_HEAD

    out_buf[0] = (x + s * g)[0:1].astype(BF16)
    db_b = ((go * s) * (sig * (1.0 + b * (1.0 - sig)))).astype(BF16)
    db_r = db_b.astype(F32)

    def ffn_bwd(t, acc):
        write_early(projection_writes + t * WRITES_PER_FFN_TILE, WRITES_PER_FFN_TILE)
        at = ffn_tile(t)
        up = up_buf[t]
        act, act_grad = _gelu_and_grad(gate_buf[t])
        dh = _nt(db_b, wd_buf[at])
        dgate = (dh * up * act_grad).astype(BF16)
        dup = (dh * act).astype(BF16)
        acc = acc + _nn(dgate, wg_buf[at]) + _nn(dup, wu_buf[at])
        for buf, col_vec, row_vec in (
            (wg_buf, dgate.astype(F32), xn_r),
            (wu_buf, dup.astype(F32), xn_r),
            (wd_buf, _bf16_rounded(act * up), db_r),
        ):
            col = _column(col_vec)
            for c in range(d_model // LANES):
                cols = slice(c * LANES, (c + 1) * LANES)
                buf[at + (cols,)] = (col * row_vec[0:1, cols]).astype(BF16)
        return acc

    dxn = jax.lax.fori_loop(0, ff_tiles, ffn_bwd, dxn)
    ffn_writes = projection_writes + ff_tiles * WRITES_PER_FFN_TILE
    dx = go + rstd * (
        dxn
        - jnp.mean(dxn, axis=-1, keepdims=True)
        - xn * jnp.mean(dxn * xn, axis=-1, keepdims=True)
    )
    dx_buf[0] = dx[0:1].astype(BF16)

    def write_attn_weights(j):
        _copy(wq_buf, dwq_hbm, wq_piece(j, ATTN_WRITE_ROWS), wq_sem).start()
        at = (all_planes, _block(j, ATTN_WRITE_ROWS))
        _copy(wo_buf, dwo_hbm, at, wo_sem).start()

    def write_ffn_weights(j):
        for _, buf, hbm, sem in ffn:
            _copy(buf, hbm, (all_planes, _block(j, FFN_ROWS)), sem).start()

    out_write = pltpu.make_async_copy(out_buf, out_hbm, x_sem)
    dx_write = pltpu.make_async_copy(dx_buf, dx_hbm, go_sem)
    out_write.start()
    dx_write.start()
    early_writes = 2 * early_groups * writes_per_cache
    assert ffn_writes <= early_writes
    write_early(ffn_writes, early_writes - ffn_writes)
    _loop(0, wo_rows // ATTN_WRITE_ROWS, write_attn_weights)
    _loop(0, ffn_pieces, write_ffn_weights)
    first_head = early_size * early_groups
    for size, groups in WRITE_GROUPS[1:]:
        write_caches(size, first_head, 0, 2 * groups * writes_per_cache)
        first_head += size * groups
    assert first_head == heads

    out_write.wait()
    dx_write.wait()
    pltpu.make_async_copy(wq_buf, dwq_hbm, wq_sem).wait()
    pltpu.make_async_copy(wo_buf, dwo_hbm, wo_sem).wait()
    for _, buf, hbm, sem in ffn:
        _copy(buf, hbm, ff_data, sem).wait()
    pltpu.make_async_copy(v_buf, dv_hbm, dv_sem).wait()
    pltpu.make_async_copy(k_buf, dk_hbm, dk_sem).wait()


@jax.jit
def pallas_recurrent_scan__gqa_block_cached__geglu_ffn__decode_kernel(
    A_x: jax.Array,
    A_k_cache: jax.Array,
    A_v_cache: jax.Array,
    A_wq: jax.Array,
    A_wo: jax.Array,
    B_x: jax.Array,
    B_w_gate: jax.Array,
    B_w_up: jax.Array,
    B_w_down: jax.Array,
    grad_out: jax.Array,
):
    del B_x
    _, heads, seq, head_dim = A_k_cache.shape
    d_model = A_x.shape[-1]
    d_attn = heads * head_dim
    d_ff = B_w_down.shape[0]
    cache = (heads, seq, head_dim)
    ff = (FFN_PLANES, d_ff // FFN_PLANES, d_model)
    ff_padded = (FFN_PLANES, pl.cdiv(ff[1], LANES) * LANES, d_model)
    ff_tiles = FFN_PLANES * ff_padded[1] // LANES
    assert ff[1] % FFN_ROWS == 0

    args = (
        A_x,
        A_k_cache.reshape(cache),
        A_v_cache.reshape(cache),
        A_wq.reshape(ATTN_PLANES, d_model // ATTN_PLANES, d_attn),
        A_wo.reshape(ATTN_PLANES, d_attn // ATTN_PLANES, d_model),
        B_w_gate.T.reshape(ff),
        B_w_up.T.reshape(ff),
        B_w_down.reshape(ff),
        grad_out,
    )
    out_like = (A_x, A_x) + args[1:8]
    hbm = pl.BlockSpec(memory_space=pltpu.HBM)

    out, dx, dk, dv, dwq, dwo, dwg_t, dwu_t, dwd = pl.pallas_call(
        _kernel,
        in_specs=[hbm] * len(args),
        out_specs=[hbm] * len(out_like),
        out_shape=[jax.ShapeDtypeStruct(a.shape, a.dtype) for a in out_like],
        scratch_shapes=[
            *(pltpu.VMEM(a.shape, BF16) for a in args[1:5]),
            *[pltpu.VMEM(ff_padded, BF16)] * 3,
            *[pltpu.VMEM(A_x.shape, BF16)] * 4,
            *[pltpu.VMEM((ff_tiles, ROWS, LANES), F32)] * 2,
            *[pltpu.VMEM((ROWS, d_attn), F32)] * 2,
            pltpu.VMEM((d_model, LANES), F32),
            *[pltpu.SemaphoreType.DMA((heads // READ_HEADS + 1,))] * 2,
            pltpu.SemaphoreType.DMA((9,)),
        ],
        compiler_params=pltpu.CompilerParams(
            vmem_limit_bytes=100 * 1024 * 1024,
            disable_bounds_checks=True,
            disable_semaphore_checks=True,
        ),
    )(*args)
    return (
        out,
        dx,
        dk.reshape(A_k_cache.shape),
        dv.reshape(A_v_cache.shape),
        dwq.reshape(A_wq.shape),
        dwo.reshape(A_wo.shape),
        dwg_t.reshape(d_ff, d_model).T,
        dwu_t.reshape(d_ff, d_model).T,
        dwd.reshape(d_ff, d_model),
    )
```
